```python
import os as _os
_os.environ.setdefault("JAX_PLATFORMS", "cpu")
import jax
import jax.numpy as jnp

def _softmax(x, axis=-1):
    return jax.nn.softmax(x, axis=axis)
def _gelu(x):
    return jax.nn.gelu(x, approximate=True)
def _silu(x):
    return jax.nn.silu(x)
def _sigmoid(x):
    return jax.nn.sigmoid(x)
def _layernorm(x, axis=-1, eps=1e-5):
    m = jnp.mean(x, axis=axis, keepdims=True)
    v = jnp.var(x, axis=axis, keepdims=True)
    return (x - m) / jnp.sqrt(v + eps)
def _scatter_add(tgt, idx, src, axis=0):
    return tgt.at[idx].add(src)
def _segment_sum(src, seg, n):
    return jax.ops.segment_sum(src, seg, n)
class _Rng:
    def __init__(self, key):
        self._k = key
    def _next(self):
        self._k, sub = jax.random.split(self._k)
        return sub
    def normal(self, shape):
        return jax.random.normal(self._next(), shape, dtype=jnp.bfloat16)
    def randint(self, lo, hi, shape):
        return jax.random.randint(self._next(), shape, lo, hi, dtype=jnp.int32)
    def uniform(self, shape, lo=0.0, hi=1.0):
        return jax.random.uniform(self._next(), shape, jnp.bfloat16, lo, hi)
    def permutation(self, n):
        return jax.random.permutation(self._next(), n)


kernel_name = 'interleave_layers__mha_block__dense_activation_mish__prompt'

def setup_inputs():
    _rng = _Rng(jax.random.key(int.from_bytes(__import__("os").urandom(4), "little")))
    _w = (lambda a: (lambda t: t.astype(jnp.bfloat16) if jnp.issubdtype(t.dtype, jnp.floating) else t)(jnp.asarray(a)))
    def _A_setup():
        B, S, D, H = 1, 2048, 512, 32
        return {
            "x": _w((lambda *s: _rng.normal(s) * 0.05)(B, S, D)),
            "wqkv": _w((lambda *s: _rng.normal(s) * 0.05)(D, 3 * D)),
            "wo": _w((lambda *s: _rng.normal(s) * 0.05)(D, D)),
        }
    _A_in = _A_setup()

    def _B_setup():
        B, S, D, F = 1, 2048, 512, 1792
        return {
            "x": _w((lambda *s: _rng.normal(s) * 0.05)(B, S, D)),
            "w1": _w((lambda *s: _rng.normal(s) * 0.4)(D, F) * (D ** -0.5)),
            "b1": _w((lambda *s: _rng.normal(s) * 0.4)(F)),
            "w2": _w((lambda *s: _rng.normal(s) * 0.4)(F, D) * (F ** -0.5)),
        }
    _B_in = _B_setup()

    return {
        "A_x": _A_in["x"],
        "A_wqkv": _A_in["wqkv"],
        "A_wo": _A_in["wo"],
        "B_x": _B_in["x"],
        "B_w1": _B_in["w1"],
        "B_b1": _B_in["b1"],
        "B_w2": _B_in["w2"],
    }

def reference(A_x, A_wqkv, A_wo, B_x, B_w1, B_b1, B_w2):
    def _A_ref(x, wqkv, wo):
        B, S, D = x.shape
        H = 32
        Dh = D // H
        qkv = (lambda x, *d: x.transpose(*d))((x @ wqkv).reshape(B, S, 3, H, Dh), 2, 0, 3, 1, 4)
        q, k, v = qkv[0], qkv[1], qkv[2]
        scores = jnp.einsum("bhqd,bhkd->bhqk", q, k) * (Dh ** -0.5)
        p = _softmax(scores, axis=-1)
        o = jnp.einsum("bhqk,bhkd->bhqd", p, v)
        return (lambda x, *d: x.transpose(*d))(o, 0, 2, 1, 3).reshape(B, S, D) @ wo

    def _B_ref(x, w1, b1, w2):
        h = jnp.einsum("bsd,df->bsf", x, w1) + b1
        sp = jnp.log1p(jnp.exp(-jnp.abs(h))) + jnp.where(h > 0, h, jnp.zeros_like(h))
        act = h * jnp.tanh(sp)
        return jnp.einsum("bsf,fd->bsd", act, w2)

    x = A_x
    x = x + _A_ref(_layernorm(x, axis=-1), A_wqkv, A_wo)
    x = x + _B_ref(_layernorm(x, axis=-1), B_w1, B_b1, B_w2)
    x = x + _A_ref(_layernorm(x, axis=-1), A_wqkv, A_wo)
    x = x + _B_ref(_layernorm(x, axis=-1), B_w1, B_b1, B_w2)
    return x
```

```python
import math
from functools import partial

import jax
import jax.numpy as jnp
from jax import lax
import jax.experimental.pallas as pl
import jax.experimental.pallas.tpu as pltpu

S, D, H, DH, F = 2048, 512, 32, 16, 1792
N_LAYERS = 2
EPS = 1e-5
TQ = 512
KC = 128
RB = 256
Q_SCALE = (DH ** -0.5) * math.log2(math.e)
F32, BF16 = jnp.float32, jnp.bfloat16
NT = (((1,), (1,)), ((), ()))
TN = (((0,), (0,)), ((), ()))


def _layernorm(x):
    m = jnp.mean(x, axis=-1, keepdims=True)
    xc = x - m
    v = jnp.mean(xc * xc, axis=-1, keepdims=True)
    return xc * lax.rsqrt(v + EPS)


def _mish(h):
    n = jnp.exp(-jnp.abs(h))
    pos = h > 0
    n2 = n + n
    nn = n * n
    num = jnp.where(pos, n2 + 1.0, nn + n2)
    den = jnp.where(pos, nn + nn + n2 + 1.0, nn + n2 + 2.0)
    return h * (num / den)


def _kernel(x_ref, wqkv_ref, wo_ref, w1_ref, b1_ref, w2_ref, o_ref,
            xs, wqvT, k_s, qT_s, vT_s, oT_s, sbuf):
    wqvT[0:D, :] = wqkv_ref[:, 0:D].astype(F32).T.astype(BF16)
    wqvT[D:2 * D, :] = wqkv_ref[:, 2 * D:3 * D].astype(F32).T.astype(BF16)

    def qkv(rows, x):
        xn = _layernorm(x).astype(BF16)
        k_s[rows, :] = jnp.dot(xn, wqkv_ref[:, D:2 * D], preferred_element_type=F32).astype(BF16)
        qv = lax.dot_general(wqvT[...], xn, NT, preferred_element_type=F32)
        qT_s[:, rows] = (qv[0:D] * Q_SCALE).astype(BF16)
        vT_s[:, rows] = qv[D:2 * D].astype(BF16)

    nq, nc, NU = S // TQ, S // KC, H * (S // TQ)
    rowh = lax.broadcasted_iota(jnp.int32, (128, 1), 0) // DH

    def idx(u):
        u = jnp.minimum(u, NU - 1)
        h = u // nq
        t = u % nq
        g = h // 8
        qs = pl.ds(pl.multiple_of(t * TQ, TQ), TQ)
        gs = pl.ds(pl.multiple_of(g * 128, 128), 128)
        hs = pl.ds(pl.multiple_of(h * DH, DH), DH)
        return h, qs, gs, hs

    def get_q(u):
        h, qs, gs, hs = idx(u)
        qT = qT_s[gs, qs]
        return jnp.where(rowh == h % 8, qT, jnp.zeros_like(qT))

    def a_dot(c, qT, gs):
        return jnp.dot(k_s[c * KC:(c + 1) * KC, gs], qT, preferred_element_type=F32)

    def a_fin(c, s, mx):
        sbuf[c * KC:(c + 1) * KC, :] = s
        for i in range(KC // 8):
            mx = jnp.maximum(mx, s[i * 8:(i + 1) * 8])
        return mx

    def attention():
        def step(u, m):
            h, qs, gs, hs = idx(u)
            _, _, gs1, _ = idx(u + 1)
            qT = get_q(u + 1)
            mx = jnp.full((8, TQ), -jnp.inf, F32)
            acc = jnp.zeros((DH, TQ), F32)
            l = jnp.zeros((8, TQ), F32)
            for c in range(nc):
                s_next = a_dot(c, qT, gs1)
                p = jnp.exp2(sbuf[c * KC:(c + 1) * KC, :] - m)
                for i in range(KC // 8):
                    l = l + p[i * 8:(i + 1) * 8]
                acc = acc + jnp.dot(vT_s[hs, c * KC:(c + 1) * KC], p.astype(BF16),
                                    preferred_element_type=F32)
                mx = a_fin(c, s_next, mx)
            oT_s[hs, qs] = (acc / jnp.sum(l, axis=0, keepdims=True)).astype(BF16)
            return jnp.max(mx, axis=0, keepdims=True)

        h, qs, gs, hs = idx(0)
        qT = get_q(0)
        mx = jnp.full((8, TQ), -jnp.inf, F32)
        for c in range(nc):
            mx = a_fin(c, a_dot(c, qT, gs), mx)
        lax.fori_loop(0, NU, step, jnp.max(mx, axis=0, keepdims=True))

    def post(rows, x):
        oT = oT_s[:, rows]
        x = x + lax.dot_general(oT, wo_ref[...], TN, preferred_element_type=F32)
        xn = _layernorm(x).astype(BF16)
        h = jnp.dot(xn, w1_ref[...], preferred_element_type=F32) + b1_ref[...].astype(F32)
        a = _mish(h).astype(BF16)
        return x + jnp.dot(a, w2_ref[...], preferred_element_type=F32)

    def rows_of(i):
        return pl.ds(pl.multiple_of(i * RB, RB), RB)

    def first(i, c):
        rows = rows_of(i)
        x = x_ref[rows, :].astype(F32)
        xs[rows, :] = x
        qkv(rows, x)
        return c

    def mid(i, c):
        rows = rows_of(i)
        x = post(rows, xs[rows, :])
        xs[rows, :] = x
        qkv(rows, x)
        return c

    def last(i, c):
        rows = rows_of(i)
        o_ref[rows, :] = post(rows, xs[rows, :]).astype(o_ref.dtype)
        return c

    lax.fori_loop(0, S // RB, first, 0)
    for layer in range(N_LAYERS):
        attention()
        lax.fori_loop(0, S // RB, mid if layer + 1 < N_LAYERS else last, 0)


@jax.jit
def pallas_interleave_layers__mha_block__dense_activation_mish__prompt_kernel(
    A_x: jax.Array,
    A_wqkv: jax.Array,
    A_wo: jax.Array,
    B_x: jax.Array,
    B_w1: jax.Array,
    B_b1: jax.Array,
    B_w2: jax.Array,
):
    del B_x
    out = pl.pallas_call(
        _kernel,
        out_shape=jax.ShapeDtypeStruct((S, D), A_x.dtype),
        scratch_shapes=[
            pltpu.VMEM((S, D), F32),
            pltpu.VMEM((2 * D, D), BF16),
            pltpu.VMEM((S, D), BF16),
            pltpu.VMEM((D, S), BF16),
            pltpu.VMEM((D, S), BF16),
            pltpu.VMEM((D, S), BF16),
            pltpu.VMEM((S, TQ), F32),
        ],
        compiler_params=pltpu.CompilerParams(vmem_limit_bytes=100 * 1024 * 1024),
    )(A_x.reshape(S, D), A_wqkv, A_wo, B_w1, B_b1.reshape(1, F), B_w2)
    return out.reshape(1, S, D)
```

```python
import math

import jax
import jax.numpy as jnp
from jax import lax
import jax.experimental.pallas as pl
import jax.experimental.pallas.tpu as pltpu

S, D, H, DH, F = 2048, 512, 32, 16, 1792
N_LAYERS = 2
EPS = 1e-5
TQ = 512
KC = 128
RB = 256
NG = D // 128
NJ = S // TQ
NC = S // KC
Q_SCALE = (DH ** -0.5) * math.log2(math.e)
F32, BF16 = jnp.float32, jnp.bfloat16
NT = (((1,), (1,)), ((), ()))
TN = (((0,), (0,)), ((), ()))


def _layernorm(x):
    m = jnp.mean(x, axis=-1, keepdims=True)
    xc = x - m
    v = jnp.mean(xc * xc, axis=-1, keepdims=True)
    return xc * lax.rsqrt(v + EPS)


def _mish(h):
    n = jnp.exp(-jnp.abs(h))
    pos = h > 0
    nn = n * n
    num = jnp.where(pos, 1.0, nn) + (n + n)
    v = jnp.where(pos, nn, 1.0)
    den = num + (v + v)
    r = pl.reciprocal(den, approx=True)
    r = r * (2.0 - den * r)
    return (h * num) * r


def _kernel(x_hbm, wqkv_hbm, wo_hbm, w1_hbm, b1_hbm, w2_hbm, o_hbm,
            k_s, st_l, w1, st_acc, b1, w2, vT_s, wqvT, qT_s, oT_s, wqkv, wo, xn_s, ostage, sbuf, xin, xs, st_mx, sems, xsems, wsems, osem):
    XP = S // 4
    x_cp = [pltpu.make_async_copy(x_hbm.at[i * XP:(i + 1) * XP, :], xin.at[i * XP:(i + 1) * XP, :], xsems.at[i])
            for i in range(4)]
    w_cp = [pltpu.make_async_copy(wqkv_hbm.at[:, i * D:(i + 1) * D], wqkv.at[:, i * D:(i + 1) * D], wsems.at[i])
            for i in range(3)]
    late = [pltpu.make_async_copy(src, dst, sems.at[i]) for i, (src, dst) in enumerate(
        [(wo_hbm, wo), (w1_hbm, w1), (b1_hbm, b1), (w2_hbm, w2)])]
    for cp in [w_cp[0], w_cp[2], x_cp[0], w_cp[1]]:
        cp.start()
    w_cp[0].wait()
    for cp in x_cp[1:]:
        cp.start()
    wqvT[0:D, :] = wqkv[:, 0:D].astype(F32).T.astype(BF16)
    w_cp[2].wait()
    wqvT[D:2 * D, :] = wqkv[:, 2 * D:3 * D].astype(F32).T.astype(BF16)
    w_cp[1].wait()

    def qkv(i, xn):
        rows = pl.ds(pl.multiple_of(i * RB, RB), RB)
        k = jnp.dot(xn, wqkv[:, D:2 * D], preferred_element_type=F32).astype(BF16)
        for g in range(NG):
            k_s[g, rows, :] = k[:, g * 128:(g + 1) * 128]
        qv = lax.dot_general(wqvT[...], xn, NT, preferred_element_type=F32)
        qT = (qv[0:D] * Q_SCALE).astype(BF16)
        vT = qv[D:2 * D].astype(BF16)
        for g in range(NG):
            qT_s[g, :, rows] = qT[g * 128:(g + 1) * 128, :]
            for cc in range(RB // KC):
                vT_s[g, i * (RB // KC) + cc] = vT[g * 128:(g + 1) * 128, cc * KC:(cc + 1) * KC]

    rowh = lax.broadcasted_iota(jnp.int32, (128, 1), 0) // DH

    def head_idx(h):
        return lax.shift_right_logical(h, 3), h & 7

    def get_q(g, hh, j):
        qT = qT_s[g, :, j * TQ:(j + 1) * TQ]
        return jnp.where(rowh == hh, qT, jnp.zeros_like(qT))

    def a_dot(c, qT, g):
        return jnp.dot(k_s[g, c * KC:(c + 1) * KC, :], qT, preferred_element_type=F32)

    def a_fin(c, j, s, mx):
        sbuf[c * KC:(c + 1) * KC, j * TQ:(j + 1) * TQ] = s
        for i in range(KC // 8):
            mx = jnp.maximum(mx, s[i * 8:(i + 1) * 8])
        return mx

    def b_chunk(c, j, m, g, hh, acc, l):
        p = jnp.exp2(sbuf[c * KC:(c + 1) * KC, j * TQ:(j + 1) * TQ] - m)
        for i in range(KC // 32):
            r0 = i * 32
            l = l + ((p[r0:r0 + 8] + p[r0 + 8:r0 + 16]) + (p[r0 + 16:r0 + 24] + p[r0 + 24:r0 + 32]))
        vrows = pl.ds(pl.multiple_of(hh * DH, DH), DH)
        acc = acc + jnp.dot(vT_s[g, c, vrows, :], p.astype(BF16), preferred_element_type=F32)
        return acc, l

    def head_step(h, ms, do_a, do_b):
        g, hh = head_idx(h)
        g1, hh1 = head_idx(h + 1)
        if do_a:
            qTs = [get_q(g1, hh1, j) for j in range(NJ)]
        mx = [jnp.full((8, TQ), -jnp.inf, F32) for _ in range(NJ)]
        acc = [jnp.zeros((DH, TQ), F32) for _ in range(NJ)]
        l = [jnp.zeros((8, TQ), F32) for _ in range(NJ)]
        for c in range(NC):
            for j in range(NJ):
                if c > 0:
                    if do_a:
                        mx[j] = st_mx[j]
                    if do_b:
                        acc[j] = st_acc[j]
                        l[j] = st_l[j]
                if do_a:
                    s = a_dot(c, qTs[j], g1)
                if do_b:
                    acc[j], l[j] = b_chunk(c, j, ms[j], g, hh, acc[j], l[j])
                if do_a:
                    mx[j] = a_fin(c, j, s, mx[j])
                if c < NC - 1:
                    if do_a:
                        st_mx[j] = mx[j]
                    if do_b:
                        st_acc[j] = acc[j]
                        st_l[j] = l[j]
        if do_b:
            vrows = pl.ds(pl.multiple_of(hh * DH, DH), DH)
            for j in range(NJ):
                o = acc[j] / jnp.sum(l[j], axis=0, keepdims=True)
                oT_s[g, vrows, j * TQ:(j + 1) * TQ] = o.astype(BF16)
        if do_a:
            return tuple(jnp.max(mx[j], axis=0, keepdims=True) for j in range(NJ))
        return ms

    def attention():
        ms = head_step(jnp.int32(-1), None, True, False)
        ms = lax.fori_loop(0, H - 1, lambda h, ms: head_step(h, ms, True, True), ms)
        head_step(jnp.int32(H - 1), ms, False, True)

    def rows_of(i):
        return pl.ds(pl.multiple_of(i * RB, RB), RB)

    def oproj(i):
        rows = rows_of(i)
        x = xs[rows, :]
        for g in range(NG):
            x = x + lax.dot_general(oT_s[g, :, rows], wo[g * 128:(g + 1) * 128, :], TN,
                                    preferred_element_type=F32)
        return x

    def ffn(xn, x):
        h = jnp.dot(xn, w1[...], preferred_element_type=F32) + b1[...].astype(F32)[None, :]
        a = _mish(h).astype(BF16)
        return x + jnp.dot(a, w2[...], preferred_element_type=F32)

    def ln(x):
        return _layernorm(x).astype(BF16)

    def ln_first(i):
        for k in (2 * i, 2 * i + 1):
            x = xin[rows_of(k), :].astype(F32)
            xs[rows_of(k), :] = x
            xn_s[rows_of(k), :] = ln(x)

    def first(i, c):
        @pl.when(i + 1 < S // RB // 2)
        def _():
            pltpu.make_async_copy(x_hbm.at[pl.ds((i + 1) * XP, XP), :], xin.at[pl.ds((i + 1) * XP, XP), :],
                                  xsems.at[i + 1]).wait()
        qkv(2 * i, xn_s[rows_of(2 * i), :])
        qkv(2 * i + 1, xn_s[rows_of(2 * i + 1), :])
        ln_first(jnp.minimum(i + 1, S // RB // 2 - 1))
        return c

    def mid(i, c):
        ia, ib = 2 * i, 2 * i + 1
        xa = oproj(ia)
        na = ln(xa)
        xb = oproj(ib)
        xa = ffn(na, xa)
        nb = ln(xb)
        xs[rows_of(ia), :] = xa
        xb = ffn(nb, xb)
        na = ln(xa)
        xs[rows_of(ib), :] = xb
        qkv(ia, na)
        nb = ln(xb)
        qkv(ib, nb)
        return c

    def last(i, c):
        ia, ib = 2 * i, 2 * i + 1
        xa = oproj(ia)
        na = ln(xa)
        xb = oproj(ib)
        xa = ffn(na, xa)
        nb = ln(xb)
        ostage[rows_of(ia), :] = xa.astype(BF16)
        pltpu.make_async_copy(ostage.at[rows_of(ia), :], o_hbm.at[rows_of(ia), :], osem).start()
        xb = ffn(nb, xb)
        ostage[rows_of(ib), :] = xb.astype(BF16)
        pltpu.make_async_copy(ostage.at[rows_of(ib), :], o_hbm.at[rows_of(ib), :], osem).start()
        return c

    x_cp[0].wait()
    ln_first(0)
    lax.fori_loop(0, S // RB // 2, first, 0)
    for cp in late:
        cp.start()

    def layer_body(layer, c):
        attention()

        @pl.when(layer == 0)
        def _():
            for cp in late:
                cp.wait()
            lax.fori_loop(0, S // RB // 2, mid, 0)

        @pl.when(layer == N_LAYERS - 1)
        def _():
            lax.fori_loop(0, S // RB // 2, last, 0)
        return c

    lax.fori_loop(0, N_LAYERS, layer_body, 0)
    pltpu.make_async_copy(ostage, o_hbm, osem).wait()


@jax.jit
def pallas_interleave_layers__mha_block__dense_activation_mish__prompt_kernel(
    A_x: jax.Array,
    A_wqkv: jax.Array,
    A_wo: jax.Array,
    B_x: jax.Array,
    B_w1: jax.Array,
    B_b1: jax.Array,
    B_w2: jax.Array,
):
    del B_x
    any_spec = pl.BlockSpec(memory_space=pl.ANY)
    out = pl.pallas_call(
        _kernel,
        out_shape=jax.ShapeDtypeStruct((S, D), A_x.dtype),
        in_specs=[any_spec] * 6,
        out_specs=any_spec,
        scratch_shapes=[
            pltpu.VMEM((NG, S, 128), BF16),
            pltpu.VMEM((NJ, 8, TQ), F32),
            pltpu.VMEM((D, F), BF16),
            pltpu.VMEM((NJ, DH, TQ), F32),
            pltpu.VMEM((F,), BF16),
            pltpu.VMEM((F, D), BF16),
            pltpu.VMEM((NG, NC, 128, KC), BF16),
            pltpu.VMEM((2 * D, D), BF16),
            pltpu.VMEM((NG, 128, S), BF16),
            pltpu.VMEM((NG, 128, S), BF16),
            pltpu.VMEM((D, 3 * D), BF16),
            pltpu.VMEM((D, D), BF16),
            pltpu.VMEM((S, D), BF16),
            pltpu.VMEM((S, D), BF16),
            pltpu.VMEM((S, S), F32),
            pltpu.VMEM((S, D), BF16),
            pltpu.VMEM((S, D), F32),
            pltpu.VMEM((NJ, 8, TQ), F32),
            pltpu.SemaphoreType.DMA((4,)),
            pltpu.SemaphoreType.DMA((4,)),
            pltpu.SemaphoreType.DMA((3,)),
            pltpu.SemaphoreType.DMA,
        ],
        compiler_params=pltpu.CompilerParams(vmem_limit_bytes=100 * 1024 * 1024),
    )(A_x.reshape(S, D), A_wqkv, A_wo, B_w1, B_b1, B_w2)
    return out.reshape(1, S, D)
```
